```python
import jax
import jax.numpy as jnp

def _softmax(x, axis=-1):
    return jax.nn.softmax(x, axis=axis)

def _gelu(x):
    return jax.nn.gelu(x, approximate=True)

def _silu(x):
    return jax.nn.silu(x)

def _sigmoid(x):
    return jax.nn.sigmoid(x)

def _layernorm(x, axis=-1, eps=1e-05):
    m = jnp.mean(x, axis=axis, keepdims=True)
    v = jnp.var(x, axis=axis, keepdims=True)
    return (x - m) / jnp.sqrt(v + eps)

def _scatter_add(tgt, idx, src, axis=0):
    return tgt.at[idx].add(src)

def _segment_sum(src, seg, n):
    return jax.ops.segment_sum(src, seg, n)

class _Rng:

    def __init__(self, key):
        self._k = key

    def _next(self):
        self._k, sub = jax.random.split(self._k)
        return sub

    def normal(self, shape):
        return jax.random.normal(self._next(), shape, dtype=jnp.bfloat16)

    def randint(self, lo, hi, shape):
        return jax.random.randint(self._next(), shape, lo, hi, dtype=jnp.int32)

    def uniform(self, shape, lo=0.0, hi=1.0):
        return jax.random.uniform(self._next(), shape, jnp.bfloat16, lo, hi)

    def permutation(self, n):
        return jax.random.permutation(self._next(), n)
kernel_name = 'standalone__conformer_conv_module__speech'

def setup_inputs():
    _rng = _Rng(jax.random.key(int.from_bytes(__import__("os").urandom(4), "little")))
    _w = lambda a: (lambda t: t.astype(jnp.bfloat16) if jnp.issubdtype(t.dtype, jnp.floating) else t)(jnp.asarray(a))
    B, T, D, K = (2, 16000, 256, 31)
    return {'x': _w((lambda *s: _rng.normal(s) * 0.05)(B, T, D)), 'w_pw1': _w((lambda *s: _rng.normal(s) * 0.05)(D, 2 * D)), 'dw': _w((lambda *s: _rng.normal(s) * 0.05)(K, D)), 'w_pw2': _w((lambda *s: _rng.normal(s) * 0.05)(D, D))}

def reference(x, w_pw1, dw, w_pw2):
    B, T, D = x.shape
    K = dw.shape[0]
    h = x @ w_pw1
    a, b = (h[..., :D].copy(), h[..., D:].copy())
    h = a * _sigmoid(b)
    pad = K // 2
    hp = jnp.pad(h, ((0, 0), (pad, pad), (0, 0)))
    out = jnp.zeros_like(h)
    for i in range(K):
        out = out + hp[:, i:i + T, :] * dw[i][None, None, :]
    return _silu(out) @ w_pw2
```

```python
import functools
import jax
import jax.numpy as jnp
import jax.experimental.pallas as pl
import jax.experimental.pallas.tpu as pltpu

BT = 3200
CH = 640
SUBN = 8

def _kernel(xp_ref, x_ref, xn_ref, w1_ref, dw_ref, w2_ref, o_ref, h_ref, u_ref, y_ref, *, nblk, K, D):
    i = pl.program_id(1)
    NC = CH // 4
    nch = BT // CH
    NH = D // 128
    w1 = w1_ref[...] * 0.5
    w2 = w2_ref[...]
    dw = dw_ref[...].astype(jnp.float32) * 0.5
    def add(a, b):
        return a if b is None else (b if a is None else a + b)
    def glu(x):
        hh = jnp.dot(x, w1, preferred_element_type=jnp.float32)
        a = hh[:, :D]
        return a * jnp.tanh(hh[:, D:]) + a
    def put(r0, v):
        for c in range(NH):
            h_ref[c, r0:r0 + v.shape[0], :] = v[:, c*128:(c+1)*128]
    def stage_a(t):
        if t == 0:
            put(0, jnp.where(i > 0, glu(xp_ref[0]), 0.0))
        put(16 + t * CH, glu(x_ref[0, t * CH:(t + 1) * CH, :]))
        if t == nch - 1:
            put(16 + BT, jnp.where(i < nblk - 1, glu(xn_ref[0]), 0.0))
            put(32 + BT, jnp.zeros((8, D), jnp.float32))
    def stage_b(t):
        n0 = 0 if t == 0 else t * NC + 8
        n = (t + 1) * NC + 8 - n0
        for c in range(NH):
            g = [h_ref[c, pl.ds(4 * n0 + p + 1, n, stride=4), :] for p in range(7)]
            p_ = g[0]-g[1]; q = g[2]-g[3]; r = g[2]-g[1]; s = g[4]-g[3]; pp = g[4]-g[5]; rp = g[6]-g[5]
            st = [p_-q, pp-q, q, r-s, rp-s, s, g[1]-g[3], g[5]-g[3], g[3]]
            for j in range(9):
                u_ref[c, j, n0:n0 + n, :] = st[j]
    W = []
    for c in range(NH):
        w = [dw[k:k+1, c*128:(c+1)*128] for k in range(K)] + [None]
        We = w[0::2]; Wo = w[1::2]; Ws = [add(a, b) for a, b in zip(We, Wo)]
        W.append([(V[0::2], V[1::2], [add(a, b) for a, b in zip(V[0::2], V[1::2])]) for V in (Ws, We, Wo)])
    def stage_c(t):
        for c in range(NH):
            for n0 in range(t * NC, (t + 1) * NC, SUBN):
                def corr(j, V, acc=None):
                    for k, v in enumerate(V):
                        if v is not None:
                            acc = add(acc, u_ref[c, j, pl.ds(n0 + k, SUBN), :] * v)
                    return acc
                def two(j0, V):
                    m = corr(j0 + 2, V[2])
                    return corr(j0, V[0], m), corr(j0 + 1, V[1], m)
                m0, m1 = two(6, W[c][0])
                a0, a1 = two(0, W[c][1])
                b0, b1 = two(3, W[c][2])
                ys = [a0 + m0, b0 + m0, a1 + m1, b1 + m1]
                for p in range(4):
                    y = ys[p]
                    y_ref[c, pl.ds(4 * n0 + p, SUBN, stride=4), :] = y * jnp.tanh(y) + y
    def stage_d(t):
        sv = jnp.concatenate([y_ref[c, t * CH:(t + 1) * CH, :] for c in range(NH)], axis=1).astype(jnp.bfloat16)
        o_ref[0, t * CH:(t + 1) * CH, :] = jnp.dot(sv, w2, preferred_element_type=jnp.float32).astype(o_ref.dtype)
    for t in range(nch + 3):
        if t < nch: stage_a(t)
        if 0 <= t - 3 < nch: stage_d(t - 3)
        if 0 <= t - 2 < nch:
            stage_b(t - 2); stage_c(t - 2)

@jax.jit
def pallas_standalone__conformer_conv_module__speech_kernel(x, w_pw1, dw, w_pw2):
    B, T, D = x.shape
    K = dw.shape[0]
    nblk = T // BT
    r16 = BT // 16
    n16 = T // 16
    return pl.pallas_call(
        functools.partial(_kernel, nblk=nblk, K=K, D=D),
        grid=(B, nblk),
        in_specs=[
            pl.BlockSpec((1, 16, D), lambda b, i: (b, jnp.maximum(i * r16 - 1, 0), 0)),
            pl.BlockSpec((1, BT, D), lambda b, i: (b, i, 0)),
            pl.BlockSpec((1, 16, D), lambda b, i: (b, jnp.minimum((i + 1) * r16, n16 - 1), 0)),
            pl.BlockSpec((D, 2 * D), lambda b, i: (0, 0)),
            pl.BlockSpec((K, D), lambda b, i: (0, 0)),
            pl.BlockSpec((D, D), lambda b, i: (0, 0)),
        ],
        out_specs=pl.BlockSpec((1, BT, D), lambda b, i: (b, i, 0)),
        out_shape=jax.ShapeDtypeStruct((B, T, D), x.dtype),
        scratch_shapes=[pltpu.VMEM((D // 128, BT + 40, 128), jnp.float32),
                        pltpu.VMEM((D // 128, 9, BT // 4 + 8, 128), jnp.float32),
                        pltpu.VMEM((D // 128, BT, 128), jnp.float32)],
        compiler_params=pltpu.CompilerParams(vmem_limit_bytes=100*2**20, dimension_semantics=("parallel", "parallel")),
    )(x, x, x, w_pw1, dw, w_pw2)
```
